```python
import jax
import jax.numpy as jnp

def _softmax(x, axis=-1):
    return jax.nn.softmax(x, axis=axis)

def _gelu(x):
    return jax.nn.gelu(x, approximate=True)

def _silu(x):
    return jax.nn.silu(x)

def _sigmoid(x):
    return jax.nn.sigmoid(x)

def _layernorm(x, axis=-1, eps=1e-05):
    m = jnp.mean(x, axis=axis, keepdims=True)
    v = jnp.var(x, axis=axis, keepdims=True)
    return (x - m) / jnp.sqrt(v + eps)

def _scatter_add(tgt, idx, src, axis=0):
    return tgt.at[idx].add(src)

def _segment_sum(src, seg, n):
    return jax.ops.segment_sum(src, seg, n)

class _Rng:

    def __init__(self, key):
        self._k = key

    def _next(self):
        self._k, sub = jax.random.split(self._k)
        return sub

    def normal(self, shape):
        return jax.random.normal(self._next(), shape, dtype=jnp.bfloat16)

    def randint(self, lo, hi, shape):
        return jax.random.randint(self._next(), shape, lo, hi, dtype=jnp.int32)

    def uniform(self, shape, lo=0.0, hi=1.0):
        return jax.random.uniform(self._next(), shape, jnp.bfloat16, lo, hi)

    def permutation(self, n):
        return jax.random.permutation(self._next(), n)
kernel_name = 'adaLN_cond__sliding_block_cached__mixer_channel_mlp__decode'

def setup_inputs():
    _rng = _Rng(jax.random.key(int.from_bytes(__import__("os").urandom(4), "little")))
    _w = lambda a: (lambda t: t.astype(jnp.bfloat16) if jnp.issubdtype(t.dtype, jnp.floating) else t)(jnp.asarray(a))

    def _A_setup():
        B, Sq, D = (8, 1, 640)
        Hq, Hkv, Sk, Dh = (32, 32, 4096, 192)
        assert Hq % Hkv == 0, (Hq, Hkv)
        return {'x': _w((lambda *s: _rng.normal(s) * 0.05)(B, Sq, D)), 'k_cache': _w((lambda *s: _rng.normal(s) * 0.05)(B, Hkv, Sk, Dh)), 'v_cache': _w((lambda *s: _rng.normal(s) * 0.05)(B, Hkv, Sk, Dh)), 'wq': _w((lambda *s: _rng.normal(s) * 0.05)(D, Hq * Dh) * D ** (-0.5)), 'wo': _w((lambda *s: _rng.normal(s) * 0.05)(Hq * Dh, D) * (Hq * Dh) ** (-0.5))}
    _A_in = _A_setup()

    def _B_setup():
        B, S, D, F = (8, 1, 640, 1536)
        return {'x': _w((lambda *s: _rng.normal(s) * 0.05)(B, S, D)), 'w1': _w((lambda *s: _rng.normal(s) * 0.05)(D, F) * D ** (-0.5)), 'b1': _w((lambda *s: _rng.normal(s) * 0.05)(F)), 'w2': _w((lambda *s: _rng.normal(s) * 0.05)(F, D) * F ** (-0.5)), 'b2': _w((lambda *s: _rng.normal(s) * 0.05)(D))}
    _B_in = _B_setup()
    return {'A_x': _A_in['x'], 'A_k_cache': _A_in['k_cache'], 'A_v_cache': _A_in['v_cache'], 'A_wq': _A_in['wq'], 'A_wo': _A_in['wo'], 'B_x': _B_in['x'], 'B_w1': _B_in['w1'], 'B_b1': _B_in['b1'], 'B_w2': _B_in['w2'], 'B_b2': _B_in['b2'], 'c': _w((lambda *s: _rng.normal(s) * 0.05)(8, 640)), 'w_mod': _w((lambda *s: _rng.normal(s) * 0.05)(640, 6 * 640) * 640 ** (-0.5))}

def reference(A_x, A_k_cache, A_v_cache, A_wq, A_wo, B_x, B_w1, B_b1, B_w2, B_b2, c, w_mod):

    def _A_ref(x, k_cache, v_cache, wq, wo):
        B, Sq, D = x.shape
        Hq, Dh = (32, 192)
        Hkv, Sk = (k_cache.shape[1], k_cache.shape[2])
        W = min(4096, max(256, Sk // 4))
        rep = Hq // Hkv
        q = (lambda x, *d: x.transpose(*d))((x @ wq).reshape(B, Sq, Hq, Dh), 0, 2, 1, 3)
        k = jnp.repeat(k_cache[:, :, Sk - W:, :], rep, axis=1)
        v = jnp.repeat(v_cache[:, :, Sk - W:, :], rep, axis=1)
        scores = jnp.einsum('bhqd,bhkd->bhqk', q, k) * Dh ** (-0.5)
        p = _softmax(scores, axis=-1)
        o = jnp.einsum('bhqk,bhkd->bhqd', p, v)
        return (lambda x, *d: x.transpose(*d))(o, 0, 2, 1, 3).reshape(B, Sq, Hq * Dh) @ wo

    def _B_ref(x, w1, b1, w2, b2):
        y = _layernorm(x, axis=-1)
        h = _gelu(jnp.einsum('bsd,df->bsf', y, w1) + b1)
        return jnp.einsum('bsf,fd->bsd', h, w2) + b2
    x = A_x
    mod = (_silu(c) @ w_mod).reshape(c.shape[0], 6, 1, -1)
    sa, ca, ga, sb, cb, gb = (mod[:, 0].copy(), mod[:, 1].copy(), mod[:, 2].copy(), mod[:, 3].copy(), mod[:, 4].copy(), mod[:, 5].copy())
    h = _layernorm(x, axis=-1) * (1 + ca) + sa
    x = x + ga * _A_ref(h, A_k_cache, A_v_cache, A_wq, A_wo)
    h = _layernorm(x, axis=-1) * (1 + cb) + sb
    x = x + gb * _B_ref(h, B_w1, B_b1, B_w2, B_b2)
    return x
```

```python
import jax
import jax.numpy as jnp
from jax import lax
import jax.experimental.pallas as pl
import jax.experimental.pallas.tpu as pltpu

_HQ, _DH = 32, 192
_PAIR = 2 * _DH
_NBUF = 8
_W2_CHUNKS = 4


def _layernorm(x, eps=1e-5):
    m = jnp.mean(x, axis=-1, keepdims=True)
    d = x - m
    v = jnp.mean(d * d, axis=-1, keepdims=True)
    return d * lax.rsqrt(v + eps)


def _dot(a, b):
    return jnp.dot(a, b, preferred_element_type=jnp.float32)


def _row_from_tiles(t, rows):
    return jnp.concatenate(
        [jnp.broadcast_to(t[j:j + 1, :], (rows, 128)) for j in range(t.shape[0])],
        axis=1)


def _kernel(c_hbm, x_hbm, wmod_hbm, wq_hbm, k_hbm, v_hbm, wo_hbm, w1_hbm,
            b1_hbm, w2_hbm, b2_hbm, out_hbm,
            c_v, x_v, b1_v, b2_v, wmod_v, wq_v, wo_v, w1_v, w2_v, kbuf, vbuf,
            out_v, sem_small, sem_mod, sem_wq, sem_wo, sem_w1, sem_w2, sem_k,
            sem_v, sem_out, *, win):
    B, D = x_v.shape
    F = w1_v.shape[1]
    sk = k_hbm.shape[2]
    npair = _HQ // 2
    nchunk = npair * B
    fc = F // _W2_CHUNKS
    bf16, f32 = jnp.bfloat16, jnp.float32
    copy = pltpu.make_async_copy

    small = [copy(s, d, sem_small.at[i]) for i, (s, d) in enumerate(
        ((c_hbm, c_v), (x_hbm, x_v), (b1_hbm, b1_v), (b2_hbm, b2_v)))]
    mod_a = copy(wmod_hbm.at[:, pl.ds(0, 2 * D)], wmod_v.at[:, pl.ds(0, 2 * D)],
                 sem_mod.at[0])
    mod_b = copy(wmod_hbm.at[:, pl.ds(2 * D, 4 * D)],
                 wmod_v.at[:, pl.ds(2 * D, 4 * D)], sem_mod.at[1])
    w1_cp = copy(w1_hbm, w1_v, sem_w1)
    w2_cp = [copy(w2_hbm.at[pl.ds(j * fc, fc)], w2_v.at[pl.ds(j * fc, fc)],
                  sem_w2.at[j]) for j in range(_W2_CHUNKS)]

    def wq_cp(p):
        col = pl.multiple_of(p * _PAIR, 128)
        return copy(wq_hbm.at[:, pl.ds(col, _PAIR)], wq_v.at[p], sem_wq.at[p])

    def wo_cp(p):
        row = pl.multiple_of(p * _PAIR, 128)
        return copy(wo_hbm.at[pl.ds(row, _PAIR)], wo_v.at[p], sem_wo.at[p])

    def kv_cp(i):
        slot = i % _NBUF
        row = pl.multiple_of((i // B) * _PAIR, 128)
        src = (i % B, pl.ds(row, _PAIR), pl.ds(sk - win, win))
        return (copy(k_hbm.at[src], kbuf.at[slot], sem_k.at[slot]),
                copy(v_hbm.at[src], vbuf.at[slot], sem_v.at[slot]))

    small[0].start()
    mod_a.start()
    for cp in small[1:]:
        cp.start()
    wq_cp(0).start()
    for i in range(_NBUF):
        for cp in kv_cp(i):
            cp.start()

    small[0].wait()
    cv = c_v[...].astype(f32)
    sc = (cv * jax.nn.sigmoid(cv)).astype(bf16)
    small[1].wait()
    x = x_v[...].astype(f32)
    xn = _layernorm(x)
    mod_a.wait()
    m = _dot(sc, wmod_v[:, 0:2 * D])
    h = (xn * (1.0 + m[:, D:2 * D]) + m[:, 0:D]).astype(bf16)

    first = lax.broadcasted_iota(jnp.int32, (B, _PAIR), 1) < _DH
    row_id = lax.broadcasted_iota(jnp.int32, (B, _PAIR), 0)
    scale = _DH ** -0.5

    def pair_body(p, attn):
        @pl.when(p + 1 < npair)
        def _():
            wq_cp(p + 1).start()
        wo_cp(p).start()
        wq_cp(p).wait()
        q = _dot(h, wq_v[p])
        q2 = jnp.concatenate(
            [jnp.where(first, q, 0.0), jnp.where(first, 0.0, q)], axis=0
        ).astype(bf16)

        def batch_body(b, o):
            i = p * B + b
            slot = i % _NBUF
            k_cp, v_cp = kv_cp(i)
            k_cp.wait()
            s = _dot(q2, kbuf[slot]) * scale
            e = jnp.exp(s - jnp.max(s, axis=-1, keepdims=True))
            inv = 1.0 / jnp.sum(e, axis=-1, keepdims=True)
            v_cp.wait()
            pv = lax.dot_general(e.astype(bf16), vbuf[slot],
                                 (((1,), (1,)), ((), ())),
                                 preferred_element_type=f32) * inv
            ob = jnp.where(first, pv[0:B], pv[B:2 * B])

            @pl.when(i + _NBUF < nchunk)
            def _():
                for cp in kv_cp(i + _NBUF):
                    cp.start()

            @pl.when(i + _NBUF == nchunk)
            def _():
                mod_b.start()
                w1_cp.start()
                for cp in w2_cp:
                    cp.start()

            return jnp.where(row_id == b, ob, o)

        o = lax.fori_loop(0, B, batch_body, jnp.zeros((B, _PAIR), f32))
        wo_cp(p).wait()
        return attn + _dot(o.astype(bf16), wo_v[p])

    attn = lax.fori_loop(0, npair, pair_body, jnp.zeros((B, D), f32))

    mod_b.wait()
    m = _dot(sc, wmod_v[:, 2 * D:6 * D])
    ga, sb, cb, gb = (m[:, j * D:(j + 1) * D] for j in range(4))
    x1 = x + ga * attn
    y = _layernorm(_layernorm(x1) * (1.0 + cb) + sb).astype(bf16)
    small[2].wait()
    small[3].wait()
    b1 = _row_from_tiles(b1_v[...].astype(f32), B)
    b2 = _row_from_tiles(b2_v[...].astype(f32), B)
    w1_cp.wait()
    u = jax.nn.gelu(_dot(y, w1_v[...]) + b1, approximate=True).astype(bf16)
    acc = b2
    for j in range(_W2_CHUNKS):
        w2_cp[j].wait()
        acc = acc + _dot(u[:, j * fc:(j + 1) * fc], w2_v[pl.ds(j * fc, fc), :])
    out_v[...] = (x1 + gb * acc).astype(out_v.dtype)
    out_cp = copy(out_v, out_hbm, sem_out)
    out_cp.start()
    out_cp.wait()


@jax.jit
def pallas_adaLN_cond__sliding_block_cached__mixer_channel_mlp__decode_kernel(
    A_x: jax.Array,
    A_k_cache: jax.Array,
    A_v_cache: jax.Array,
    A_wq: jax.Array,
    A_wo: jax.Array,
    B_x: jax.Array,
    B_w1: jax.Array,
    B_b1: jax.Array,
    B_w2: jax.Array,
    B_b2: jax.Array,
    c: jax.Array,
    w_mod: jax.Array,
):
    del B_x
    B, Sq, D = A_x.shape
    _, Hkv, Sk, Dh = A_k_cache.shape
    F = B_w1.shape[1]
    assert (Sq, Hkv, Dh) == (1, _HQ, _DH)
    win = min(4096, max(256, Sk // 4))
    npair = _HQ // 2

    kt = jnp.swapaxes(A_k_cache, 2, 3).reshape(B, Hkv * Dh, Sk)
    vt = jnp.swapaxes(A_v_cache, 2, 3).reshape(B, Hkv * Dh, Sk)

    bf16 = jnp.bfloat16
    vmem, dma = pltpu.VMEM, pltpu.SemaphoreType.DMA
    hbm = pl.BlockSpec(memory_space=pltpu.HBM)

    def kernel(*refs):
        _kernel(*refs, win=win)

    out = pl.pallas_call(
        kernel,
        out_shape=jax.ShapeDtypeStruct((B, D), A_x.dtype),
        in_specs=[hbm] * 11,
        out_specs=hbm,
        scratch_shapes=[
            vmem((B, D), bf16), vmem((B, D), bf16),
            vmem((F // 128, 128), bf16), vmem((D // 128, 128), bf16),
            vmem((D, 6 * D), bf16),
            vmem((npair, D, _PAIR), bf16), vmem((npair, _PAIR, D), bf16),
            vmem((D, F), bf16), vmem((F, D), bf16),
            vmem((_NBUF, _PAIR, win), bf16), vmem((_NBUF, _PAIR, win), bf16),
            vmem((B, D), A_x.dtype),
            dma((4,)), dma((2,)), dma((npair,)), dma((npair,)), dma(()),
            dma((_W2_CHUNKS,)), dma((_NBUF,)), dma((_NBUF,)), dma(()),
        ],
        compiler_params=pltpu.CompilerParams(
            vmem_limit_bytes=100 * 1024 * 1024),
    )(c, A_x.reshape(B, D), w_mod, A_wq, kt, vt, A_wo, B_w1,
      B_b1.reshape(F // 128, 128), B_w2, B_b2.reshape(D // 128, 128))
    return out.reshape(B, Sq, D)
```

```python
import itertools

import jax
import jax.numpy as jnp
from jax import lax
import jax.experimental.pallas as pl
import jax.experimental.pallas.tpu as pltpu

_HQ, _DH = 32, 192
_PAIR = 2 * _DH
_AHEAD = 2
_NBUF = 4
_KV_DIGITS = ((16, 3), (1, 2), (4, 2), (2, 2), (8, 2))
_WQ_PARTS = 3
_WQ_WAYS = 4
_WO_PARTS = 4
_WO_WAYS = 6
_W2_PARTS = 4
_KV_ORDER = tuple(
    sum(w * d for (w, _), d in zip(reversed(_KV_DIGITS), t))
    for t in itertools.product(*[range(r) for _, r in reversed(_KV_DIGITS)]))


def _layernorm(x, eps=1e-5):
    m = jnp.mean(x, axis=-1, keepdims=True)
    d = x - m
    v = jnp.mean(d * d, axis=-1, keepdims=True)
    return d * lax.rsqrt(v + eps)


def _dot(a, b):
    return jnp.dot(a, b, preferred_element_type=jnp.float32)


def _row_from_tiles(t, rows):
    return jnp.concatenate(
        [jnp.broadcast_to(t[j:j + 1, :], (rows, 128)) for j in range(t.shape[0])],
        axis=1)


def _stream(src, dst, sem, row0, nrows, cols, piece, ways, steps=None):
    per = nrows // (piece * ways)
    assert per * piece * ways == nrows
    lo, hi = steps or (0, per)

    def body(i, carry):
        for w in range(ways):
            r = pl.multiple_of(row0 + (w * per + i) * piece, 8)
            sl = (pl.ds(r, piece), cols)
            pltpu.make_async_copy(src.at[sl], dst.at[sl], sem).start(priority=w % 2)
        return carry

    lax.fori_loop(lo, hi, body, None)


def _await(window, sem):
    pltpu.make_async_copy(window, window, sem).wait()


def _kernel(c_hbm, x_hbm, wmod_hbm, wq_hbm, k_hbm, v_hbm, wo_hbm, w1_hbm,
            b1_hbm, w2_hbm, b2_hbm, out_hbm,
            c_v, x_v, b1_v, b2_v, wmod_v, wq_v, wo_v, w1_v, w2_v, kbuf, vbuf,
            q_v, o_v, out_v, sem_small, sem_mod, sem_wq, sem_wo, sem_w1, sem_w2,
            sem_k, sem_v, sem_out, *, win):
    B, D = x_v.shape
    F = w1_v.shape[1]
    sk = k_hbm.shape[2]
    npair = _HQ // 2
    nchunk = npair * B
    qc = _HQ * _DH // _WQ_PARTS
    oc = _HQ * _DH // _WO_PARTS
    fc = F // _W2_PARTS
    half = len(_KV_ORDER) // 2
    bf16, f32 = jnp.bfloat16, jnp.float32
    everything = slice(None)

    def start_mod(j):
        _stream(wmod_hbm, wmod_v, sem_mod.at[j], 0, D, pl.ds(2 * D * j, 2 * D), 8, 4)

    def mod(j):
        cols = pl.ds(2 * D * j, 2 * D)
        _await(wmod_v.at[:, cols], sem_mod.at[j])
        m = _dot(sc, wmod_v[:, cols])
        return m[:, 0:D], m[:, D:2 * D]

    def start_wq(j):
        _stream(wq_hbm, wq_v, sem_wq.at[j], 0, D, pl.ds(qc * j, qc), 8, _WQ_WAYS)

    def start_wo(j, quarter=None):
        per = oc // (16 * _WO_WAYS)
        steps = None if quarter is None else (quarter * per // 4, (quarter + 1) * per // 4)
        _stream(wo_hbm, wo_v, sem_wo.at[j], oc * j, oc, everything, 16, _WO_WAYS, steps)

    def start_kv(i, quarter):
        src, dst, sem = ((k_hbm, kbuf, sem_k), (v_hbm, vbuf, sem_v))[quarter // 2]
        slot = lax.rem(i, _NBUF)
        b, row0 = lax.rem(i, B), lax.div(i, B) * _PAIR
        for n, g in enumerate(_KV_ORDER[(quarter % 2) * half:][:half]):
            r = pl.multiple_of(row0 + 8 * g, 8)
            pltpu.make_async_copy(
                src.at[b, pl.ds(r, 8), pl.ds(sk - win, win)],
                dst.at[slot, pl.ds(8 * g, 8)], sem.at[slot]).start(priority=n % 2)

    def start_next(i, quarter):
        @pl.when(i < nchunk)
        def _():
            start_kv(i, quarter)

        for j in range(_AHEAD):
            @pl.when(i == nchunk + j)
            def _():
                start_wo(j, quarter)

    small = [pltpu.make_async_copy(s, d, sem_small.at[i]) for i, (s, d) in enumerate(
        ((c_hbm, c_v), (x_hbm, x_v), (b1_hbm, b1_v), (b2_hbm, b2_v)))]
    for cp in small:
        cp.start()
    start_mod(0)
    start_wq(0)
    for cp in small:
        cp.wait()
    cv = c_v[...].astype(f32)
    sc = (cv * jax.nn.sigmoid(cv)).astype(bf16)
    x = x_v[...].astype(f32)
    xn = _layernorm(x)
    start_wq(1)
    sa, ca = mod(0)
    h = (xn * (1.0 + ca) + sa).astype(bf16)

    lane = lax.broadcasted_iota(jnp.int32, (B, 128), 1)

    def project_q(j):
        cols = pl.ds(qc * j, qc)
        _await(wq_v.at[:, cols], sem_wq.at[j])
        q = _dot(h, wq_v[:, cols])
        for t in range(qc // 128):
            p, u = divmod(j * qc // 128 + t, 3)
            qt = q[:, 128 * t:128 * (t + 1)]
            first = lane < _DH - 128 * u
            q_v[p, :, 128 * u:128 * (u + 1)] = jnp.concatenate(
                [jnp.where(first, qt, 0.0), jnp.where(first, 0.0, qt)],
                axis=0).astype(bf16)

    for j in range(2, _WQ_PARTS):
        start_wq(j)
        project_q(j - 2)
    for quarter in range(4):
        start_kv(jnp.int32(0), quarter)
    project_q(_WQ_PARTS - 2)
    for quarter in range(4):
        start_kv(jnp.int32(1), quarter)
    project_q(_WQ_PARTS - 1)

    first = lax.broadcasted_iota(jnp.int32, (B, _PAIR), 1) < _DH
    row_id = lax.broadcasted_iota(jnp.int32, (B, _PAIR), 0)
    scale = _DH ** -0.5

    def pair_body(p, carry):
        def batch_body(b, o):
            i = p * B + b
            slot = lax.rem(i, _NBUF)
            start_next(i + _AHEAD, 0)
            _await(kbuf.at[slot], sem_k.at[slot])
            s = _dot(q_v[p], kbuf[slot]) * scale
            start_next(i + _AHEAD, 1)
            e = jnp.exp(s - jnp.max(s, axis=-1, keepdims=True))
            inv = 1.0 / jnp.sum(e, axis=-1, keepdims=True)
            start_next(i + _AHEAD, 2)
            _await(vbuf.at[slot], sem_v.at[slot])
            pv = lax.dot_general(e.astype(bf16), vbuf[slot],
                                 (((1,), (1,)), ((), ())),
                                 preferred_element_type=f32) * inv
            start_next(i + _AHEAD, 3)
            return jnp.where(row_id == b, jnp.where(first, pv[0:B], pv[B:2 * B]), o)

        o_v[p] = lax.fori_loop(0, B, batch_body, jnp.zeros((B, _PAIR), f32))
        return carry

    lax.fori_loop(0, npair, pair_body, None)

    def project_o(j):
        _await(wo_v.at[pl.ds(oc * j, oc)], sem_wo.at[j])
        n = oc // _PAIR
        o = jnp.concatenate([o_v[j * n + t] for t in range(n)], axis=1)
        return _dot(o.astype(bf16), wo_v[pl.ds(oc * j, oc), :])

    attn = None
    for j in range(_WO_PARTS):
        if j + _AHEAD < _WO_PARTS:
            start_wo(j + _AHEAD)
        else:
            start_mod(j + _AHEAD - _WO_PARTS + 1)
        attn = project_o(j) if attn is None else attn + project_o(j)

    _stream(w1_hbm, w1_v, sem_w1, 0, D, everything, 8, 4)
    ga, sb = mod(1)
    x1 = x + ga * attn
    x1n = _layernorm(x1)
    for j in range(_W2_PARTS):
        _stream(w2_hbm, w2_v, sem_w2.at[j], fc * j, fc, everything, 16, 6)
    cb, gb = mod(2)
    y = _layernorm(x1n * (1.0 + cb) + sb).astype(bf16)
    b1 = _row_from_tiles(b1_v[...].astype(f32), B)
    acc = _row_from_tiles(b2_v[...].astype(f32), B)
    _await(w1_v, sem_w1)
    u = jax.nn.gelu(_dot(y, w1_v[...]) + b1, approximate=True).astype(bf16)
    for j in range(_W2_PARTS):
        _await(w2_v.at[pl.ds(fc * j, fc)], sem_w2.at[j])
        acc = acc + _dot(u[:, j * fc:(j + 1) * fc], w2_v[pl.ds(j * fc, fc), :])
    out_v[...] = (x1 + gb * acc).astype(out_v.dtype)
    out_cp = pltpu.make_async_copy(out_v, out_hbm, sem_out)
    out_cp.start()
    out_cp.wait()


@jax.jit
def pallas_adaLN_cond__sliding_block_cached__mixer_channel_mlp__decode_kernel(
    A_x: jax.Array,
    A_k_cache: jax.Array,
    A_v_cache: jax.Array,
    A_wq: jax.Array,
    A_wo: jax.Array,
    B_x: jax.Array,
    B_w1: jax.Array,
    B_b1: jax.Array,
    B_w2: jax.Array,
    B_b2: jax.Array,
    c: jax.Array,
    w_mod: jax.Array,
):
    del B_x
    B, Sq, D = A_x.shape
    _, Hkv, Sk, Dh = A_k_cache.shape
    F = B_w1.shape[1]
    assert (Sq, Hkv, Dh) == (1, _HQ, _DH)
    win = min(4096, max(256, Sk // 4))
    npair = _HQ // 2

    kt = jnp.swapaxes(A_k_cache, 2, 3).reshape(B, Hkv * Dh, Sk)
    vt = jnp.swapaxes(A_v_cache, 2, 3).reshape(B, Hkv * Dh, Sk)

    bf16 = jnp.bfloat16
    vmem, dma = pltpu.VMEM, pltpu.SemaphoreType.DMA
    hbm = pl.BlockSpec(memory_space=pltpu.HBM)

    def kernel(*refs):
        _kernel(*refs, win=win)

    out = pl.pallas_call(
        kernel,
        out_shape=jax.ShapeDtypeStruct((B, D), A_x.dtype),
        in_specs=[hbm] * 11,
        out_specs=hbm,
        scratch_shapes=[
            vmem((B, D), bf16), vmem((B, D), bf16),
            vmem((F // 128, 128), bf16), vmem((D // 128, 128), bf16),
            vmem((D, 6 * D), bf16),
            vmem((D, Hkv * Dh), bf16), vmem((Hkv * Dh, D), bf16),
            vmem((D, F), bf16), vmem((F, D), bf16),
            vmem((_NBUF, _PAIR, win), bf16), vmem((_NBUF, _PAIR, win), bf16),
            vmem((npair, 2 * B, _PAIR), bf16), vmem((npair, B, _PAIR), jnp.float32),
            vmem((B, D), A_x.dtype),
            dma((4,)), dma((3,)), dma((_WQ_PARTS,)), dma((_WO_PARTS,)), dma(()),
            dma((_W2_PARTS,)), dma((_NBUF,)), dma((_NBUF,)), dma(()),
        ],
        compiler_params=pltpu.CompilerParams(
            vmem_limit_bytes=64 * 1024 * 1024),
    )(c, A_x.reshape(B, D), w_mod, A_wq, kt, vt, A_wo, B_w1,
      B_b1.reshape(F // 128, 128), B_w2, B_b2.reshape(D // 128, 128))
    return out.reshape(B, Sq, D)
```

```python
import itertools

import jax
import jax.numpy as jnp
from jax import lax
import jax.experimental.pallas as pl
import jax.experimental.pallas.tpu as pltpu

_HQ, _DH = 32, 192
_PAIR = 2 * _DH
_AHEAD = 2
_NBUF = 4
_KV_DIGITS = ((16, 3), (1, 2), (2, 2), (4, 2), (8, 2))
_WQ_PARTS = 3
_WQ_WAYS = 10
_WO_PARTS = 4
_WO_WAYS = 6
_W2_PARTS = 2
_KV_ORDER = tuple(
    sum(w * d for (w, _), d in zip(reversed(_KV_DIGITS), t))
    for t in itertools.product(*[range(r) for _, r in reversed(_KV_DIGITS)]))
_KV_PRIO = '0011'
_KV_PIECES = tuple((a, g, int(_KV_PRIO[(2 * n + a) % len(_KV_PRIO)]))
                   for n, g in enumerate(_KV_ORDER) for a in range(2))


def _layernorm(x, eps=1e-5):
    m = jnp.mean(x, axis=-1, keepdims=True)
    d = x - m
    v = jnp.mean(d * d, axis=-1, keepdims=True)
    return d * lax.rsqrt(v + eps)


def _dot(a, b):
    return jnp.dot(a, b, preferred_element_type=jnp.float32)


def _row_from_tiles(t, rows):
    return jnp.concatenate(
        [jnp.broadcast_to(t[j:j + 1, :], (rows, 128)) for j in range(t.shape[0])],
        axis=1)


def _stream(src, dst, sem, row0, nrows, cols, piece, ways, steps=None):
    per = nrows // (piece * ways)
    assert per * piece * ways == nrows
    lo, hi = steps or (0, per)

    def body(i, carry):
        for w in range(ways):
            r = pl.multiple_of(row0 + (w * per + i) * piece, 8)
            sl = (pl.ds(r, piece), cols)
            pltpu.make_async_copy(src.at[sl], dst.at[sl], sem).start(priority=w % 2)
        return carry

    lax.fori_loop(lo, hi, body, None)


def _await(window, sem):
    pltpu.make_async_copy(window, window, sem).wait()


def _kernel(c_hbm, x_hbm, wmod_hbm, wq_hbm, k_hbm, v_hbm, wo_hbm, w1_hbm,
            b1_hbm, w2_hbm, b2_hbm, out_hbm,
            c_v, x_v, b1_v, b2_v, wmod_v, wq_v, wo_v, w1_v, w2_v, kv_v,
            q_v, o_v, out_v, sem_small, sem_mod, sem_wq, sem_wo, sem_w1, sem_w2,
            sem_kv, sem_out, *, win):
    B, D = x_v.shape
    F = w1_v.shape[1]
    sk = k_hbm.shape[2]
    npair = _HQ // 2
    nchunk = npair * B
    qc = _HQ * _DH // _WQ_PARTS
    oc = _HQ * _DH // _WO_PARTS
    fc = F // _W2_PARTS
    half = len(_KV_ORDER) // 2
    bf16, f32 = jnp.bfloat16, jnp.float32
    everything = slice(None)

    mod_cols = (pl.ds(0, 2 * D), pl.ds(2 * D, 4 * D))

    def start_mod(j):
        _stream(wmod_hbm, wmod_v, sem_mod.at[j], 0, D, mod_cols[j], 8, (16, 8)[j])

    def mod(j):
        m = _dot(sc, wmod_v[:, pl.ds(2 * D * j, 2 * D)])
        return m[:, 0:D], m[:, D:2 * D]

    def start_wq(j):
        _stream(wq_hbm, wq_v, sem_wq.at[j], 0, D, pl.ds(qc * j, qc), 8, _WQ_WAYS)

    wo_steps = _HQ * _DH // (16 * _WO_WAYS)
    wo_quarter = half // _WO_WAYS

    def start_wo(lo, hi):
        _stream(wo_hbm, wo_v, sem_wo, 0, _HQ * _DH, everything, 16, _WO_WAYS, (lo, hi))

    def start_kv(i, quarter):
        slot = lax.rem(i, _NBUF)
        b, row0 = lax.rem(i, B), lax.div(i, B) * _PAIR
        for a, g, prio in _KV_PIECES[quarter * half:][:half]:
            r = pl.multiple_of(row0 + 8 * g, 8)
            pltpu.make_async_copy(
                (k_hbm, v_hbm)[a].at[b, pl.ds(r, 8), pl.ds(sk - win, win)],
                kv_v.at[slot, a, pl.ds(8 * g, 8)], sem_kv.at[slot]).start(priority=prio)

    def start_next(i, quarter):
        @pl.when(i < nchunk)
        def _():
            start_kv(i, quarter)

        @pl.when(i >= nchunk)
        def _():
            lo = ((i - nchunk) * 4 + quarter) * wo_quarter
            start_wo(lo, lo + wo_quarter)

    small = [pltpu.make_async_copy(s, d, sem_small.at[i]) for i, (s, d) in enumerate(
        ((c_hbm, c_v), (x_hbm, x_v), (b1_hbm, b1_v), (b2_hbm, b2_v)))]
    for cp in small:
        cp.start()
    start_mod(0)
    start_wq(0)
    for cp in small:
        cp.wait()
    cv = c_v[...].astype(f32)
    sc = (cv * jax.nn.sigmoid(cv)).astype(bf16)
    x = x_v[...].astype(f32)
    xn = _layernorm(x)
    start_wq(1)
    _await(wmod_v.at[:, mod_cols[0]], sem_mod.at[0])
    sa, ca = mod(0)
    h = (xn * (1.0 + ca) + sa).astype(bf16)

    lane = lax.broadcasted_iota(jnp.int32, (B, 128), 1)

    def project_q(j):
        cols = pl.ds(qc * j, qc)
        _await(wq_v.at[:, cols], sem_wq.at[j])
        q = _dot(h, wq_v[:, cols])
        for t in range(qc // 128):
            p, u = divmod(j * qc // 128 + t, 3)
            qt = q[:, 128 * t:128 * (t + 1)]
            first = lane < _DH - 128 * u
            q_v[p, :, 128 * u:128 * (u + 1)] = jnp.concatenate(
                [jnp.where(first, qt, 0.0), jnp.where(first, 0.0, qt)],
                axis=0).astype(bf16)

    for j in range(2, _WQ_PARTS):
        start_wq(j)
        project_q(j - 2)
    def start_chunk(i, carry):
        for quarter in range(4):
            start_kv(i, quarter)
        return carry

    lax.fori_loop(0, 1, start_chunk, None)
    project_q(_WQ_PARTS - 2)
    lax.fori_loop(1, _AHEAD, start_chunk, None)
    project_q(_WQ_PARTS - 1)

    first = lax.broadcasted_iota(jnp.int32, (B, _PAIR), 1) < _DH
    row_id = lax.broadcasted_iota(jnp.int32, (B, _PAIR), 0)
    scale = _DH ** -0.5

    def pair_body(p, carry):
        def batch_body(b, o):
            i = p * B + b
            slot = lax.rem(i, _NBUF)
            start_next(i + _AHEAD, 0)
            _await(kv_v.at[slot], sem_kv.at[slot])
            s = _dot(q_v[p], kv_v[slot, 0]) * scale
            start_next(i + _AHEAD, 1)
            e = jnp.exp(s - jnp.max(s, axis=-1, keepdims=True))
            inv = 1.0 / jnp.sum(e, axis=-1, keepdims=True)
            start_next(i + _AHEAD, 2)
            pv = lax.dot_general(e.astype(bf16), kv_v[slot, 1],
                                 (((1,), (1,)), ((), ())),
                                 preferred_element_type=f32) * inv
            start_next(i + _AHEAD, 3)
            return jnp.where(row_id == b, jnp.where(first, pv[0:B], pv[B:2 * B]), o)

        o_v[p] = lax.fori_loop(0, B, batch_body, jnp.zeros((B, _PAIR), f32))
        return carry

    lax.fori_loop(0, npair, pair_body, None)

    def project_o(j):
        n = oc // _PAIR
        o = jnp.concatenate([o_v[j * n + t] for t in range(n)], axis=1)
        return _dot(o.astype(bf16), wo_v[pl.ds(oc * j, oc), :])

    start_wo(4 * _AHEAD * wo_quarter, wo_steps)
    start_mod(1)
    _await(wo_v, sem_wo)
    attn = project_o(0) + project_o(1)
    _stream(w1_hbm, w1_v, sem_w1, 0, D, everything, 8, 8)
    attn = attn + project_o(2) + project_o(3)
    _stream(w2_hbm, w2_v, sem_w2.at[0], 0, fc, everything, 16, 4)
    _await(wmod_v.at[:, mod_cols[1]], sem_mod.at[1])
    ga, sb = mod(1)
    x1 = x + ga * attn
    x1n = _layernorm(x1)
    for j in range(1, _W2_PARTS):
        _stream(w2_hbm, w2_v, sem_w2.at[j], fc * j, fc, everything, 16, 4)
    cb, gb = mod(2)
    y = _layernorm(x1n * (1.0 + cb) + sb).astype(bf16)
    b1 = _row_from_tiles(b1_v[...].astype(f32), B)
    acc = _row_from_tiles(b2_v[...].astype(f32), B)
    _await(w1_v, sem_w1)
    u = jax.nn.gelu(_dot(y, w1_v[...]) + b1, approximate=True).astype(bf16)
    for j in range(_W2_PARTS):
        _await(w2_v.at[pl.ds(fc * j, fc)], sem_w2.at[j])
        acc = acc + _dot(u[:, j * fc:(j + 1) * fc], w2_v[pl.ds(j * fc, fc), :])
    out_v[...] = (x1 + gb * acc).astype(out_v.dtype)
    out_cp = pltpu.make_async_copy(out_v, out_hbm, sem_out)
    out_cp.start()
    out_cp.wait()


@jax.jit
def pallas_adaLN_cond__sliding_block_cached__mixer_channel_mlp__decode_kernel(
    A_x: jax.Array,
    A_k_cache: jax.Array,
    A_v_cache: jax.Array,
    A_wq: jax.Array,
    A_wo: jax.Array,
    B_x: jax.Array,
    B_w1: jax.Array,
    B_b1: jax.Array,
    B_w2: jax.Array,
    B_b2: jax.Array,
    c: jax.Array,
    w_mod: jax.Array,
):
    del B_x
    B, Sq, D = A_x.shape
    _, Hkv, Sk, Dh = A_k_cache.shape
    F = B_w1.shape[1]
    assert (Sq, Hkv, Dh) == (1, _HQ, _DH)
    win = min(4096, max(256, Sk // 4))
    npair = _HQ // 2

    kt = jnp.swapaxes(A_k_cache, 2, 3).reshape(B, Hkv * Dh, Sk)
    vt = jnp.swapaxes(A_v_cache, 2, 3).reshape(B, Hkv * Dh, Sk)

    bf16 = jnp.bfloat16
    vmem, dma = pltpu.VMEM, pltpu.SemaphoreType.DMA
    hbm = pl.BlockSpec(memory_space=pltpu.HBM)

    def kernel(*refs):
        _kernel(*refs, win=win)

    out = pl.pallas_call(
        kernel,
        out_shape=jax.ShapeDtypeStruct((B, D), A_x.dtype),
        in_specs=[hbm] * 11,
        out_specs=hbm,
        scratch_shapes=[
            vmem((B, D), bf16), vmem((B, D), bf16),
            vmem((F // 128, 128), bf16), vmem((D // 128, 128), bf16),
            vmem((D, 6 * D), bf16),
            vmem((D, Hkv * Dh), bf16), vmem((Hkv * Dh, D), bf16),
            vmem((D, F), bf16), vmem((F, D), bf16),
            vmem((_NBUF, 2, _PAIR, win), bf16),
            vmem((npair, 2 * B, _PAIR), bf16), vmem((npair, B, _PAIR), jnp.float32),
            vmem((B, D), A_x.dtype),
            dma((4,)), dma((2,)), dma((_WQ_PARTS,)), dma(()), dma(()),
            dma((_W2_PARTS,)), dma((_NBUF,)), dma(()),
        ],
        compiler_params=pltpu.CompilerParams(
            vmem_limit_bytes=64 * 1024 * 1024),
    )(c, A_x.reshape(B, D), w_mod, A_wq, kt, vt, A_wo, B_w1,
      B_b1.reshape(F // 128, 128), B_w2, B_b2.reshape(D // 128, 128))
    return out.reshape(B, Sq, D)
```

```python
import jax
import jax.numpy as jnp
from jax import lax
import jax.experimental.pallas as pl
import jax.experimental.pallas.tpu as pltpu

_HQ, _DH = 32, 192
_PAIR = 2 * _DH
_AHEAD = 2
_NBUF = 4
_WQ_PARTS = 3
_WO_PARTS = 4
_WO_PIECE, _WO_WAYS = 16, 6
_W2_SPLIT = (3, 2, 1)

_KV_PIECES = tuple((kv, 16 * hi + lo, (lo + hi) % 2)
                   for lo in range(16) for hi in range(3) for kv in range(2))


def _layernorm(x, eps=1e-5):
    m = jnp.mean(x, axis=-1, keepdims=True)
    d = x - m
    v = jnp.mean(d * d, axis=-1, keepdims=True)
    return d * lax.rsqrt(v + eps)


def _dot(a, b):
    return jnp.dot(a, b, preferred_element_type=jnp.float32)


def _row_from_tiles(t, rows):
    return jnp.concatenate(
        [jnp.broadcast_to(t[j:j + 1, :], (rows, 128)) for j in range(t.shape[0])],
        axis=1)


def _stream(src, dst, sem, rows, cols, piece, ways, steps=None):
    nsteps = rows.size // (piece * ways)
    assert nsteps * piece * ways == rows.size

    def body(i, carry):
        for w in range(ways):
            r = pl.multiple_of(rows.start + (w * nsteps + i) * piece, 8)
            for n, col in enumerate(cols):
                window = (pl.ds(r, piece), col)
                pltpu.make_async_copy(src.at[window], dst.at[window], sem).start(
                    priority=(w * len(cols) + n) % 2)
        return carry

    lax.fori_loop(*(steps or (0, nsteps)), body, None)


def _await(window, sem):
    pltpu.make_async_copy(window, window, sem).wait()


def _kernel(c_hbm, x_hbm, wmod_hbm, wq_hbm, k_hbm, v_hbm, wo_hbm, w1_hbm,
            b1_hbm, w2_hbm, b2_hbm, out_hbm,
            c_v, x_v, b1_v, b2_v, wmod_v, wq_v, wo_v, w1_v, w2_v, kv_v,
            q_v, o_v, out_v, sems, small_sem):
    B, D = x_v.shape
    F = w1_v.shape[1]
    sk, win = k_hbm.shape[2], kv_v.shape[3]
    npair = _HQ // 2
    nchunk = npair * B
    issue_points = 4
    per_point = len(_KV_PIECES) // issue_points
    wq_cols = _HQ * _DH // _WQ_PARTS
    wo_rows = _HQ * _DH // _WO_PARTS
    wo_steps = _HQ * _DH // (_WO_PIECE * _WO_WAYS)
    wo_per_point = per_point // _WO_WAYS
    unit = F // sum(_W2_SPLIT)
    w2_rows = [pl.ds(unit * sum(_W2_SPLIT[:j]), unit * n)
               for j, n in enumerate(_W2_SPLIT)]
    full = (slice(None),)
    bf16, f32 = jnp.bfloat16, jnp.float32

    def start_wq(j):
        _stream(wq_hbm, wq_v, sems.at[1 + j], pl.ds(0, D),
                (pl.ds(wq_cols * j, wq_cols),), 8, 10)

    def start_wo(lo, hi):
        _stream(wo_hbm, wo_v, sems.at[0], pl.ds(0, _HQ * _DH), full,
                _WO_PIECE, _WO_WAYS, (lo, hi))

    def start_w2(j):
        _stream(w2_hbm, w2_v, sems.at[(2 + j) % _NBUF], w2_rows[j], full, 16, 4)

    def start_kv(i, point):
        slot = lax.rem(i, _NBUF)
        b, row0 = lax.rem(i, B), lax.div(i, B) * _PAIR
        for kv, g, queue in _KV_PIECES[point * per_point:][:per_point]:
            r = pl.multiple_of(row0 + 8 * g, 8)
            pltpu.make_async_copy(
                (k_hbm, v_hbm)[kv].at[b, pl.ds(r, 8), pl.ds(sk - win, win)],
                kv_v.at[slot, kv, pl.ds(8 * g, 8)],
                sems.at[slot]).start(priority=queue)

    def start_next(i, point):
        @pl.when(i < nchunk)
        def _():
            start_kv(i, point)

        @pl.when(i >= nchunk)
        def _():
            lo = ((i - nchunk) * issue_points + point) * wo_per_point
            start_wo(lo, lo + wo_per_point)

    _stream(wmod_hbm, wmod_v, sems.at[0], pl.ds(0, D),
            (pl.ds(0, 3 * D), pl.ds(3 * D, 3 * D)), 8, 5)
    small = [pltpu.make_async_copy(src, dst, small_sem) for src, dst in
             ((c_hbm, c_v), (x_hbm, x_v), (b1_hbm, b1_v), (b2_hbm, b2_v))]
    for cp in small:
        cp.start()
    start_wq(0)
    start_wq(1)
    for cp in small:
        cp.wait()
    _await(wmod_v, sems.at[0])
    cv = c_v[...].astype(f32)
    silu_c = (cv * jax.nn.sigmoid(cv)).astype(bf16)

    def mod(j):
        m = _dot(silu_c, wmod_v[:, pl.ds(2 * D * j, 2 * D)])
        return m[:, 0:D], m[:, D:2 * D]

    x = x_v[...].astype(f32)
    sa, ca = mod(0)
    h = (_layernorm(x) * (1.0 + ca) + sa).astype(bf16)
    lane = lax.broadcasted_iota(jnp.int32, (B, 128), 1)

    def project_q(j):
        cols = pl.ds(wq_cols * j, wq_cols)
        _await(wq_v.at[:, cols], sems.at[1 + j])
        q = _dot(h, wq_v[:, cols])
        for t in range(wq_cols // 128):
            p, u = divmod(wq_cols * j // 128 + t, _PAIR // 128)
            qt = q[:, 128 * t:128 * (t + 1)]
            first = lane < _DH - 128 * u
            q_v[p, :, 128 * u:128 * (u + 1)] = jnp.concatenate(
                [jnp.where(first, qt, 0.0), jnp.where(first, 0.0, qt)],
                axis=0).astype(bf16)

    start_wq(2)
    project_q(0)
    for i in range(_AHEAD):
        for point in range(issue_points):
            start_kv(jnp.int32(i), point)
        project_q(1 + i)

    first_head = lax.broadcasted_iota(jnp.int32, (B, _PAIR), 1) < _DH
    row_id = lax.broadcasted_iota(jnp.int32, (B, _PAIR), 0)

    def pair_body(p, carry):
        def batch_body(b, o):
            i = p * B + b
            slot = lax.rem(i, _NBUF)
            start_next(i + _AHEAD, 0)
            _await(kv_v.at[slot], sems.at[slot])
            s = _dot(q_v[p], kv_v[slot, 0]) * _DH ** -0.5
            start_next(i + _AHEAD, 1)
            e = jnp.exp(s - jnp.max(s, axis=-1, keepdims=True))
            inv_sum = 1.0 / jnp.sum(e, axis=-1, keepdims=True)
            start_next(i + _AHEAD, 2)
            pv = lax.dot_general(e.astype(bf16), kv_v[slot, 1],
                                 (((1,), (1,)), ((), ())),
                                 preferred_element_type=f32) * inv_sum
            start_next(i + _AHEAD, 3)
            return jnp.where(row_id == b,
                             jnp.where(first_head, pv[0:B], pv[B:2 * B]), o)

        o_v[p] = lax.fori_loop(0, B, batch_body, jnp.zeros((B, _PAIR), f32))
        return carry

    lax.fori_loop(0, npair, pair_body, None)

    def project_o(j):
        n = wo_rows // _PAIR
        o = jnp.concatenate([o_v[j * n + t] for t in range(n)], axis=1)
        return _dot(o.astype(bf16), wo_v[pl.ds(wo_rows * j, wo_rows), :])

    wo_issued = _AHEAD * issue_points * wo_per_point
    wo_half = (wo_issued + wo_steps) // 2
    start_wo(wo_issued, wo_half)
    ga, sb = mod(1)
    start_wo(wo_half, wo_steps)
    cb, gb = mod(2)
    _stream(w1_hbm, w1_v, sems.at[1], pl.ds(0, D), full, 8, 8)
    _await(wo_v, sems.at[0])
    attn = project_o(0) + project_o(1)
    start_w2(0)
    x1 = x + ga * (attn + project_o(2) + project_o(3))
    y = _layernorm(_layernorm(x1) * (1.0 + cb) + sb).astype(bf16)
    for j in range(1, len(w2_rows)):
        start_w2(j)
    b1 = _row_from_tiles(b1_v[...].astype(f32), B)
    mlp = _row_from_tiles(b2_v[...].astype(f32), B)
    _await(w1_v, sems.at[1])
    u = jax.nn.gelu(_dot(y, w1_v[...]) + b1, approximate=True).astype(bf16)
    for j, rows in enumerate(w2_rows):
        _await(w2_v.at[rows], sems.at[(2 + j) % _NBUF])
        mlp = mlp + _dot(u[:, rows.start:rows.start + rows.size], w2_v[rows, :])
    out_v[...] = (x1 + gb * mlp).astype(out_v.dtype)
    out_cp = pltpu.make_async_copy(out_v, out_hbm, small_sem)
    out_cp.start()
    out_cp.wait()


@jax.jit
def pallas_adaLN_cond__sliding_block_cached__mixer_channel_mlp__decode_kernel(
    A_x: jax.Array,
    A_k_cache: jax.Array,
    A_v_cache: jax.Array,
    A_wq: jax.Array,
    A_wo: jax.Array,
    B_x: jax.Array,
    B_w1: jax.Array,
    B_b1: jax.Array,
    B_w2: jax.Array,
    B_b2: jax.Array,
    c: jax.Array,
    w_mod: jax.Array,
):
    del B_x
    B, Sq, D = A_x.shape
    _, Hkv, Sk, Dh = A_k_cache.shape
    F = B_w1.shape[1]
    assert (Sq, Hkv, Dh) == (1, _HQ, _DH)
    win = min(4096, max(256, Sk // 4))
    npair = _HQ // 2

    kt = jnp.swapaxes(A_k_cache, 2, 3).reshape(B, Hkv * Dh, Sk)
    vt = jnp.swapaxes(A_v_cache, 2, 3).reshape(B, Hkv * Dh, Sk)

    bf16 = jnp.bfloat16
    vmem = pltpu.VMEM
    hbm = pl.BlockSpec(memory_space=pltpu.HBM)

    out = pl.pallas_call(
        _kernel,
        out_shape=jax.ShapeDtypeStruct((B, D), A_x.dtype),
        in_specs=[hbm] * 11,
        out_specs=hbm,
        scratch_shapes=[
            vmem((B, D), bf16), vmem((B, D), bf16),
            vmem((F // 128, 128), bf16), vmem((D // 128, 128), bf16),
            vmem((D, 6 * D), bf16),
            vmem((D, Hkv * Dh), bf16), vmem((Hkv * Dh, D), bf16),
            vmem((D, F), bf16), vmem((F, D), bf16),
            vmem((_NBUF, 2, _PAIR, win), bf16),
            vmem((npair, 2 * B, _PAIR), bf16),
            vmem((npair, B, _PAIR), jnp.float32),
            vmem((B, D), A_x.dtype),
            pltpu.SemaphoreType.DMA((_NBUF,)), pltpu.SemaphoreType.DMA(()),
        ],
        compiler_params=pltpu.CompilerParams(
            vmem_limit_bytes=64 * 1024 * 1024),
    )(c, A_x.reshape(B, D), w_mod, A_wq, kt, vt, A_wo, B_w1,
      B_b1.reshape(F // 128, 128), B_w2, B_b2.reshape(D // 128, 128))
    return out.reshape(B, Sq, D)
```
